```python
import os as _os
_os.environ.setdefault("JAX_PLATFORMS", "cpu")
import jax
import jax.numpy as jnp

def _softmax(x, axis=-1):
    return jax.nn.softmax(x, axis=axis)
def _gelu(x):
    return jax.nn.gelu(x, approximate=True)
def _silu(x):
    return jax.nn.silu(x)
def _sigmoid(x):
    return jax.nn.sigmoid(x)
def _layernorm(x, axis=-1, eps=1e-5):
    m = jnp.mean(x, axis=axis, keepdims=True)
    v = jnp.var(x, axis=axis, keepdims=True)
    return (x - m) / jnp.sqrt(v + eps)
def _scatter_add(tgt, idx, src, axis=0):
    return tgt.at[idx].add(src)
def _segment_sum(src, seg, n):
    return jax.ops.segment_sum(src, seg, n)
class _Rng:
    def __init__(self, key):
        self._k = key
    def _next(self):
        self._k, sub = jax.random.split(self._k)
        return sub
    def normal(self, shape):
        return jax.random.normal(self._next(), shape, dtype=jnp.bfloat16)
    def randint(self, lo, hi, shape):
        return jax.random.randint(self._next(), shape, lo, hi, dtype=jnp.int32)
    def uniform(self, shape, lo=0.0, hi=1.0):
        return jax.random.uniform(self._next(), shape, jnp.bfloat16, lo, hi)
    def permutation(self, n):
        return jax.random.permutation(self._next(), n)


kernel_name = 'concat_heads__gqa_block_cached__gqa_block_cached__decode'

def setup_inputs():
    _rng = _Rng(jax.random.key(int.from_bytes(__import__("os").urandom(4), "little")))
    _w = (lambda a: (lambda t: t.astype(jnp.bfloat16) if jnp.issubdtype(t.dtype, jnp.floating) else t)(jnp.asarray(a)))
    def _A_setup():
        B, Sq, D = 2, 1, 576
        Hq, Hkv, Sk, Dh = 32, 16, 4096, 128
        assert Hq % Hkv == 0, (Hq, Hkv)
        return {
            "x": _w((lambda *s: _rng.normal(s) * 0.8)(B, Sq, D)),
            "k_cache": _w((lambda *s: _rng.normal(s) * 0.8)(B, Hkv, Sk, Dh)),
            "v_cache": _w((lambda *s: _rng.normal(s) * 0.05)(B, Hkv, Sk, Dh)),
            "wq": _w((lambda *s: _rng.normal(s) * 0.8)(D, Hq * Dh) * (D ** -0.5)),
            "wo": _w((lambda *s: _rng.normal(s) * 0.05)(Hq * Dh, D) * ((Hq * Dh) ** -0.5)),
        }
    _A_in = _A_setup()

    def _B_setup():
        B, Sq, D = 2, 1, 576
        Hq, Hkv, Sk, Dh = 32, 16, 4096, 128
        assert Hq % Hkv == 0, (Hq, Hkv)
        return {
            "x": _w((lambda *s: _rng.normal(s) * 0.8)(B, Sq, D)),
            "k_cache": _w((lambda *s: _rng.normal(s) * 0.8)(B, Hkv, Sk, Dh)),
            "v_cache": _w((lambda *s: _rng.normal(s) * 0.05)(B, Hkv, Sk, Dh)),
            "wq": _w((lambda *s: _rng.normal(s) * 0.8)(D, Hq * Dh) * (D ** -0.5)),
            "wo": _w((lambda *s: _rng.normal(s) * 0.05)(Hq * Dh, D) * ((Hq * Dh) ** -0.5)),
        }
    _B_in = _B_setup()

    return {
        "A_x": _A_in["x"],
        "A_k_cache": _A_in["k_cache"],
        "A_v_cache": _A_in["v_cache"],
        "A_wq": _A_in["wq"],
        "A_wo": _A_in["wo"],
        "B_x": _B_in["x"],
        "B_k_cache": _B_in["k_cache"],
        "B_v_cache": _B_in["v_cache"],
        "B_wq": _B_in["wq"],
        "B_wo": _B_in["wo"],
    }

def reference(A_x, A_k_cache, A_v_cache, A_wq, A_wo, B_x, B_k_cache, B_v_cache, B_wq, B_wo):
    def _A_ref(x, k_cache, v_cache, wq, wo):
        B, Sq, D = x.shape
        Hq, Dh = 32, 128
        Hkv = k_cache.shape[1]
        rep = Hq // Hkv
        q = (lambda x, *d: x.transpose(*d))((x @ wq).reshape(B, Sq, Hq, Dh), 0, 2, 1, 3)
        k = jnp.repeat(k_cache, rep, axis=1)
        v = jnp.repeat(v_cache, rep, axis=1)
        scores = jnp.einsum("bhqd,bhkd->bhqk", q, k) * (Dh ** -0.5)
        p = _softmax(scores, axis=-1)
        o = jnp.einsum("bhqk,bhkd->bhqd", p, v)
        return (lambda x, *d: x.transpose(*d))(o, 0, 2, 1, 3).reshape(B, Sq, Hq * Dh) @ wo

    def _B_ref(x, k_cache, v_cache, wq, wo):
        B, Sq, D = x.shape
        Hq, Dh = 32, 128
        Hkv = k_cache.shape[1]
        rep = Hq // Hkv
        q = (lambda x, *d: x.transpose(*d))((x @ wq).reshape(B, Sq, Hq, Dh), 0, 2, 1, 3)
        k = jnp.repeat(k_cache, rep, axis=1)
        v = jnp.repeat(v_cache, rep, axis=1)
        scores = jnp.einsum("bhqd,bhkd->bhqk", q, k) * (Dh ** -0.5)
        p = _softmax(scores, axis=-1)
        o = jnp.einsum("bhqk,bhkd->bhqd", p, v)
        return (lambda x, *d: x.transpose(*d))(o, 0, 2, 1, 3).reshape(B, Sq, Hq * Dh) @ wo

    a = _A_ref(A_x, A_k_cache, A_v_cache, A_wq, A_wo)
    b = _B_ref(B_x, B_k_cache, B_v_cache, B_wq, B_wo)
    return jnp.concatenate([a, b], axis=-1)
```

```python
import functools

import jax
import jax.numpy as jnp
from jax import lax
from jax.experimental import pallas as pl
from jax.experimental.pallas import tpu as pltpu

B, D, HQ, HKV, SK, DH = 2, 576, 32, 16, 4096, 128
HD = HQ * DH
NI = B * HKV
C = 128
H = C // 2
NP = SK // C
G = 4
S = B * G
PG = NP // S
SLOTS = 3
AHEAD = S + 2
STREAMS = ((0, 0), (0, 1), (2, 1), (2, 0), (3, 0), (3, 1), (1, 1), (1, 0))
PHASE = (0, 1)
HALF = HD // 2
R1, R2 = 768, 1024
K3 = 3072
NT = (((1,), (1,)), ((), ()))


def _aligned(i, n):
    return i if isinstance(i, int) else pl.multiple_of(i, n)


def _wait_all(view, sem):
    pltpu.make_async_copy(view, view, sem).wait()


def _weight_pieces(br, half, r8):
    if not PHASE[br]:
        return [(r8, half * HALF, 0, HALF)]
    q = HALF // 2
    if half == 0:
        return [(r8, q, 0, HALF)]
    return [(r8, 3 * q, 0, q), ((r8 + 1) % 8, 0, q, q)]


def _kernel(ax, ak, av, awq, awo, bx, bk, bv, bwq, bwo, o_ref,
            kv_buf, wq_buf, wo_buf, q_scr, o_scr, acc, x_buf, w_sem, kv_sem):

    def request_cache(br, g):
        unit = g // S
        slot = unit % SLOTS
        base = (unit - br * (HKV // G)) * (G * SK)
        p0 = (g % S) * PG
        srcs = ((ak, av), (bk, bv))[br]

        def start(a, b, *pieces):
            for r0, n in pieces:
                pltpu.make_async_copy(srcs[a].at[pl.ds(_aligned(base + b * HKV * SK + r0, H), n)],
                                      kv_buf.at[slot, a, pl.ds(_aligned(b * G * SK + r0, H), n)],
                                      kv_sem.at[slot]).start(priority=a)

        for p in range(PG):
            r = (p0 + p) * C + PHASE[br] * H
            wraps = PHASE[br] and p == PG - 1
            last = H if wraps else C
            views = [(srcs[a].at[pl.ds(_aligned(base + r, H), (HKV + G - 1) * SK + last)],
                      kv_buf.at[slot, a, pl.ds(_aligned(r, H), (S - 1) * SK + last)]) for a in range(2)]
            for h, b in STREAMS:
                for a, (src, dst) in enumerate(views):
                    if wraps and h == G - 1:
                        pl.when(r + C <= SK)(functools.partial(start, a, b, (r + h * SK, C)))
                        pl.when(r + C > SK)(functools.partial(start, a, b, (G * SK - H, H), (0, H)))
                    else:
                        pltpu.make_async_copy(src.at[pl.ds((b * HKV + h) * SK, C)],
                                              dst.at[pl.ds((b * G + h) * SK, C)],
                                              kv_sem.at[slot]).start(priority=a)

    def wo_chunk(s, half, r8, sem):
        br = int(64 * s >= D)
        return [pltpu.make_async_copy(
                    (awo, bwo)[br].at[pl.ds(_aligned(64 * s - br * D + 8 * rb, 8), 8), pl.ds(c, n)],
                    wo_buf.at[pl.ds(_aligned(64 * s + 8 * rb, 8), 8), pl.ds(half * HALF + dc, n)],
                    w_sem.at[sem])
                for rb, c, dc, n in _weight_pieces(br, half, r8)]

    def start_wo_chunk(s, half, r8, sem):
        for copy in wo_chunk(s, half, r8, sem):
            copy.start(priority=s % 2)

    def request_wo(half, lo, hi):
        def body(r8, _):
            for s in range((R1 if half else R2) // 64):
                start_wo_chunk(s, half, r8, half)
        lax.fori_loop(lo, hi, body, None)

    for p in range(16):
        for s in range(D // 64):
            for br, src in enumerate((awq, bwq)):
                for rb, c, _, n in _weight_pieces(br, p % 2, p // 2):
                    idx = (pl.ds(64 * s + 8 * rb, 8), pl.ds(c, n))
                    pltpu.make_async_copy(src.at[idx], wq_buf.at[(br,) + idx], w_sem.at[0]).start(priority=br)
        if p == 0:
            for br, src in enumerate((ax, bx)):
                pltpu.make_async_copy(src, x_buf.at[br], w_sem.at[1]).start(priority=br)
    lax.fori_loop(0, AHEAD - 8, lambda g, _: request_cache(0, g), None)
    _wait_all(x_buf, w_sem.at[1])
    _wait_all(wq_buf, w_sem.at[0])

    row = lax.broadcasted_iota(jnp.int32, (8, DH), 0)
    row_x = lax.broadcasted_iota(jnp.int32, (8, D), 0)

    def project_q(j, _):
        request_cache(0, j + AHEAD - 8)
        for br in range(2):
            x = x_buf[br].astype(jnp.float32)
            x = jnp.where(row_x % 2 == 0, x[0:1], x[1:2]).astype(jnp.bfloat16)
            q = jnp.dot(x, wq_buf[br, :, pl.ds(_aligned(j * 4 * DH, 4 * DH), 4 * DH)],
                        preferred_element_type=jnp.float32)
            for t in range(2):
                c = 2 * t * DH
                q_scr[br * HKV + 2 * j + t] = jnp.where(
                    (row // 2) % 2 == 0, q[:, c:c + DH], q[:, c + DH:c + 2 * DH])
    lax.fori_loop(0, HKV // 2, project_q, None)

    def attend(request, i, _):
        slot = (i // S) % SLOTS

        @pl.when(i % S == 0)
        def _():
            _wait_all(kv_buf.at[slot], kv_sem.at[slot])

        request(i)
        rows = pl.ds(_aligned((i % S) * SK, SK), SK)
        q = q_scr[(i // S) * G + i % G].astype(jnp.bfloat16)
        s = lax.dot_general(q, kv_buf[slot, 0, rows], NT, preferred_element_type=jnp.float32)
        s = s * (DH ** -0.5)
        p = jnp.exp(s - jnp.max(s, axis=1, keepdims=True))
        l = jnp.sum(p, axis=1, keepdims=True)
        o = jnp.dot(p.astype(jnp.bfloat16), kv_buf[slot, 1, rows], preferred_element_type=jnp.float32)
        o_scr[i] = o / l

    def request_tail(i):
        j = i - (2 * NI - AHEAD)
        lo = jnp.where(j == 0, 0, jnp.where(j == 1, 4, j + 4))
        hi = jnp.where(j == 0, 4, j + 5)
        request_wo(0, jnp.minimum(lo, 8), jnp.minimum(hi, 8))
        request_wo(1, jnp.maximum(lo, 8) - 8, jnp.maximum(hi, 8) - 8)

    lax.fori_loop(0, NI - AHEAD,
                  functools.partial(attend, lambda i: request_cache(0, i + AHEAD)), None)
    lax.fori_loop(NI - AHEAD, 2 * NI - AHEAD,
                  functools.partial(attend, lambda i: request_cache(1, i + AHEAD)), None)
    lax.fori_loop(2 * NI - AHEAD, 2 * NI, functools.partial(attend, request_tail), None)

    request_wo(1, AHEAD + 4 - 8, 8)

    def request_mid(r8, _):
        for s in range(R1 // 64 + 1, R2 // 64, 2):
            start_wo_chunk(s, 1, r8, 2)
    lax.fori_loop(0, 8, request_mid, None)
    paced = [(s, r8) for r8 in range(8) for s in range(R1 // 64, R2 // 64, 2)]

    def feed(n):
        for s, r8 in paced[:n]:
            start_wo_chunk(s, 1, r8, 2)
        del paced[:n]

    heads = []
    for br in range(2):
        tiles = []
        for h in range(HKV):
            i = br * NI + (h // G) * S + h % G
            even = jnp.where(row % 2 == 0, o_scr[i], o_scr[i + G])
            tiles += [even, pltpu.roll(even, 6, 0)]
        heads.append(tiles)
    rotated = [t[8 * ph:] + t[:8 * ph] for t, ph in zip(heads, PHASE)]
    o_ab = jnp.concatenate(
        [jnp.concatenate(ab, axis=0).astype(jnp.bfloat16) for ab in zip(*rotated)], axis=1)
    o_b = jnp.concatenate(heads[1], axis=1).astype(jnp.bfloat16)

    def project_o(lhs, r0, r1, c0, c1):
        return lax.dot_general(lhs[:, c0:c1], wo_buf[r0:r1, c0:c1], NT, preferred_element_type=jnp.float32)

    def finish(r0, r1):
        r = acc[:, r0:r1] + project_o(o_ab, r0, r1, HALF, HD)
        col = r0 + lax.broadcasted_iota(jnp.int32, (8, r1 - r0), 1)
        o_ref[:, r0:r1] = jnp.where(col < D, r[0:8], r[8:16])[0:B].astype(o_ref.dtype)

    _wait_all(wo_buf.at[pl.ds(0, R2), pl.ds(0, HALF)], w_sem.at[0])
    for r in range(0, R2, 256):
        acc[:, r:r + 256] = project_o(o_ab, r, r + 256, 0, HALF)
        feed(2)

    for sem, c0, c1 in ((3, 0, K3), (4, K3, HD)):
        def request_last(r8, _, sem=sem, cols=pl.ds(c0, c1 - c0)):
            pltpu.make_async_copy(bwo.at[pl.ds(_aligned(R2 - D + 8 * r8, 8), 8), cols],
                                  wo_buf.at[pl.ds(_aligned(R2 + 8 * r8, 8), 8), cols],
                                  w_sem.at[sem]).start(priority=1)
        lax.fori_loop(0, (2 * D - R2) // 8, request_last, None)

    chunks = [(s, r8) for r8 in range(8) for s in range(R1 // 64)]
    for n, (s, r8) in enumerate(chunks):
        if n >= len(chunks) - 32 and n % 4 == 0:
            feed(1)
        for copy in wo_chunk(s, 1, r8, 1):
            copy.wait()
    feed(len(paced))
    for r in range(0, R1, 256):
        finish(r, r + 256)
    _wait_all(wo_buf.at[pl.ds(R1, R2 - R1), pl.ds(HALF, HALF)], w_sem.at[2])
    finish(R1, R2)
    _wait_all(wo_buf.at[pl.ds(R2, 2 * D - R2), pl.ds(0, K3)], w_sem.at[3])
    acc[0:8, R2:] = project_o(o_b, R2, 2 * D, 0, K3)
    _wait_all(wo_buf.at[pl.ds(R2, 2 * D - R2), pl.ds(K3, HD - K3)], w_sem.at[4])
    o_ref[:, R2:] = (acc[0:8, R2:] + project_o(o_b, R2, 2 * D, K3, HD))[0:B].astype(o_ref.dtype)


@jax.jit
def pallas_concat_heads__gqa_block_cached__gqa_block_cached__decode_kernel(
    A_x: jax.Array,
    A_k_cache: jax.Array,
    A_v_cache: jax.Array,
    A_wq: jax.Array,
    A_wo: jax.Array,
    B_x: jax.Array,
    B_k_cache: jax.Array,
    B_v_cache: jax.Array,
    B_wq: jax.Array,
    B_wo: jax.Array,
):
    def rows(cache):
        return cache.reshape(NI * SK, DH)

    out = pl.pallas_call(
        _kernel,
        out_shape=jax.ShapeDtypeStruct((B, 2 * D), A_x.dtype),
        in_specs=[pl.BlockSpec(memory_space=pltpu.MemorySpace.HBM)] * 10,
        scratch_shapes=[
            pltpu.VMEM((SLOTS, 2, S * SK, DH), jnp.bfloat16),
            pltpu.VMEM((2, D, HD), jnp.bfloat16),
            pltpu.VMEM((2 * D, HD), jnp.bfloat16),
            pltpu.VMEM((2 * HKV, 8, DH), jnp.float32),
            pltpu.VMEM((2 * NI, 8, DH), jnp.float32),
            pltpu.VMEM((16, 2 * D), jnp.float32),
            pltpu.VMEM((2, B, D), jnp.bfloat16),
            pltpu.SemaphoreType.DMA((5,)),
            pltpu.SemaphoreType.DMA((SLOTS,)),
        ],
        compiler_params=pltpu.CompilerParams(
            vmem_limit_bytes=100 * 2**20,
            disable_bounds_checks=True,
            disable_semaphore_checks=True,
        ),
    )(A_x.reshape(B, D), rows(A_k_cache), rows(A_v_cache), A_wq, A_wo.T,
      B_x.reshape(B, D), rows(B_k_cache), rows(B_v_cache), B_wq, B_wo.T)
    return out.reshape(B, 1, 2 * D)
```
